```python
import jax
import jax.numpy as jnp

def _softmax(x, axis=-1):
    return jax.nn.softmax(x, axis=axis)
def _gelu(x):
    return jax.nn.gelu(x, approximate=True)
def _silu(x):
    return jax.nn.silu(x)
def _sigmoid(x):
    return jax.nn.sigmoid(x)
def _layernorm(x, axis=-1, eps=1e-5):
    m = jnp.mean(x, axis=axis, keepdims=True)
    v = jnp.var(x, axis=axis, keepdims=True)
    return (x - m) / jnp.sqrt(v + eps)
def _scatter_add(tgt, idx, src, axis=0):
    return tgt.at[idx].add(src)
def _segment_sum(src, seg, n):
    return jax.ops.segment_sum(src, seg, n)
class _Rng:
    def __init__(self, key):
        self._k = key
    def _next(self):
        self._k, sub = jax.random.split(self._k)
        return sub
    def normal(self, shape):
        return jax.random.normal(self._next(), shape, dtype=jnp.bfloat16)
    def randint(self, lo, hi, shape):
        return jax.random.randint(self._next(), shape, lo, hi, dtype=jnp.int32)
    def uniform(self, shape, lo=0.0, hi=1.0):
        return jax.random.uniform(self._next(), shape, jnp.bfloat16, lo, hi)
    def permutation(self, n):
        return jax.random.permutation(self._next(), n)


kernel_name = 'sequential_preLN__mha_block_cached__moe_arch_mod__decode'

def setup_inputs():
    _rng = _Rng(jax.random.key(int.from_bytes(__import__("os").urandom(4), "little")))
    _w = (lambda a: (lambda t: t.astype(jnp.bfloat16) if jnp.issubdtype(t.dtype, jnp.floating) else t)(jnp.asarray(a)))
    def _A_setup():
        B, Sq, D = 4, 1, 640
        H, Sk, Dh = 32, 8192, 192
        return {
            "x": _w((lambda *s: _rng.normal(s) * 0.05)(B, Sq, D)),
            "k_cache": _w((lambda *s: _rng.normal(s) * 0.05)(B, H, Sk, Dh)),
            "v_cache": _w((lambda *s: _rng.normal(s) * 0.05)(B, H, Sk, Dh)),
            "wq": _w((lambda *s: _rng.normal(s) * 0.05)(D, H * Dh) * (D ** -0.5)),
            "wo": _w((lambda *s: _rng.normal(s) * 0.05)(H * Dh, D) * ((H * Dh) ** -0.5)),
        }
    _A_in = _A_setup()

    def _B_setup():
        B, S, D, F, C = 4, 1, 640, 1536, 1
        return {
            "x": _w((lambda *s: _rng.normal(s) * 0.05)(B, S, D)),
            "w_r": _w((lambda *s: _rng.normal(s) * 0.05)(D)),
            "w_gate": _w((lambda *s: _rng.normal(s) * 0.05)(D, F)),
            "w_up": _w((lambda *s: _rng.normal(s) * 0.05)(D, F)),
            "w_down": _w((lambda *s: _rng.normal(s) * 0.05)(F, D)),
        }
    _B_in = _B_setup()

    return {
        "A_x": _A_in["x"],
        "A_k_cache": _A_in["k_cache"],
        "A_v_cache": _A_in["v_cache"],
        "A_wq": _A_in["wq"],
        "A_wo": _A_in["wo"],
        "B_x": _B_in["x"],
        "B_w_r": _B_in["w_r"],
        "B_w_gate": _B_in["w_gate"],
        "B_w_up": _B_in["w_up"],
        "B_w_down": _B_in["w_down"],
    }

def reference(A_x, A_k_cache, A_v_cache, A_wq, A_wo, B_x, B_w_r, B_w_gate, B_w_up, B_w_down):
    def _A_ref(x, k_cache, v_cache, wq, wo):
        B, Sq, D = x.shape
        H, Dh = 32, 192
        q = (lambda x, *d: x.transpose(*d))((x @ wq).reshape(B, Sq, H, Dh), 0, 2, 1, 3)
        scores = jnp.einsum("bhqd,bhkd->bhqk", q, k_cache) * (Dh ** -0.5)
        p = _softmax(scores, axis=-1)
        o = jnp.einsum("bhqk,bhkd->bhqd", p, v_cache)
        return (lambda x, *d: x.transpose(*d))(o, 0, 2, 1, 3).reshape(B, Sq, H * Dh) @ wo

    def _B_ref(x, w_r, w_gate, w_up, w_down):
        B, S, D = x.shape
        C = 1
        r = x @ w_r
        idx = jnp.argsort(-r, axis=-1)[:, :C]
        idx_e = jnp.repeat(idx.reshape(B, C, 1), D, axis=2)
        x_sel = jnp.take_along_axis(x, idx_e, axis=1)
        g = _silu(x_sel @ w_gate)
        u = x_sel @ w_up
        y = (g * u) @ w_down
        r_sel = _sigmoid(jnp.take_along_axis(r, idx, axis=1))
        y = y * r_sel.reshape(B, C, 1)
        b_off = (jnp.arange(B) * S).reshape(B, 1)
        flat_idx = (idx + b_off).reshape(B * C)
        zero = (x * 0.0).reshape(B * S, D)
        upd = _scatter_add(zero, flat_idx, y.reshape(B * C, D), axis=0)
        return x + upd.reshape(B, S, D)

    x = A_x
    h = x + _A_ref(_layernorm(x, axis=-1), A_k_cache, A_v_cache, A_wq, A_wo)
    h2 = h + _B_ref(_layernorm(h, axis=-1), B_w_r, B_w_gate, B_w_up, B_w_down)
    return h2
```

```python
import jax
import jax.numpy as jnp
from jax import lax
from jax.experimental import pallas as pl
from jax.experimental.pallas import tpu as pltpu

_EPS = 1e-5
_ROWS = 8


def _layernorm(x):
    m = jnp.mean(x, axis=-1, keepdims=True)
    d = x - m
    v = jnp.mean(d * d, axis=-1, keepdims=True)
    return d / jnp.sqrt(v + _EPS)


def _mm(a, b):
    return jnp.dot(a, b, preferred_element_type=jnp.float32)


def _kernel(x_hbm, kt_hbm, vt_hbm, wq_hbm, wo_hbm, wr_hbm, wg_hbm, wu_hbm, wd_hbm,
            out_ref,
            x_v, wq_v, wo_v, wr_v, wg_v, wu_v, wd_v, k_buf, v_buf, q_s, xpad_s,
            k_sem, v_sem, w_sem):
    f32, bf16 = jnp.float32, jnp.bfloat16
    B, H, Dh, _ = kt_hbm.shape
    D = x_hbm.shape[1]
    scale = float(Dh) ** -0.5

    def k_copy(b, h):
        return pltpu.make_async_copy(kt_hbm.at[b, h], k_buf.at[b], k_sem.at[b])

    def v_copy(b, h):
        return pltpu.make_async_copy(vt_hbm.at[b, h], v_buf.at[b], v_sem.at[b])

    x_cp = pltpu.make_async_copy(x_hbm, x_v, w_sem.at[0])
    wq_cp = pltpu.make_async_copy(wq_hbm, wq_v, w_sem.at[1])
    wo_cp = pltpu.make_async_copy(wo_hbm, wo_v, w_sem.at[2])
    wr_cp = pltpu.make_async_copy(wr_hbm, wr_v, w_sem.at[3])
    wg_cp = pltpu.make_async_copy(wg_hbm, wg_v, w_sem.at[4])
    wu_cp = pltpu.make_async_copy(wu_hbm, wu_v, w_sem.at[5])
    wd_cp = pltpu.make_async_copy(wd_hbm, wd_v, w_sem.at[6])

    wq_cp.start()
    x_cp.start()
    for b in range(B):
        k_copy(b, 0).start()
        v_copy(b, 0).start()
    wo_cp.start()
    wr_cp.start()

    x_cp.wait()
    xpad_s[...] = jnp.zeros((_ROWS, D), f32)
    xpad_s[0:B, :] = x_v[...].astype(f32)
    x = xpad_s[...]
    xn = _layernorm(x).astype(bf16)
    wq_cp.wait()
    for hp in range(H // 2):
        q2 = _mm(xn, wq_v[:, hp * 2 * Dh:(hp + 1) * 2 * Dh])
        q_s[2 * hp] = q2[:, :Dh]
        q_s[2 * hp + 1] = q2[:, Dh:]

    row = lax.broadcasted_iota(jnp.int32, (_ROWS, Dh), 0)

    def head(h, attn):
        q = q_s[h].astype(bf16)
        o_h = jnp.zeros((_ROWS, Dh), f32)
        for b in range(B):
            k_copy(b, h).wait()
            s = _mm(q, k_buf[b]) * scale

            @pl.when(h + 1 < H)
            def _():
                k_copy(b, h + 1).start()

            p = jnp.exp(s - jnp.max(s, axis=-1, keepdims=True))
            l = jnp.sum(p, axis=-1, keepdims=True)
            v_copy(b, h).wait()
            o = lax.dot_general(p.astype(bf16), v_buf[b], (((1,), (1,)), ((), ())),
                                preferred_element_type=f32)

            @pl.when(h + 1 < H)
            def _():
                v_copy(b, h + 1).start()

            o_h = jnp.where(row == b, o / l, o_h)

        @pl.when(h == 0)
        def _():
            wo_cp.wait()
            wr_cp.wait()

        @pl.when(h == H - 2)
        def _():
            wg_cp.start()
            wu_cp.start()
            wd_cp.start()

        w = wo_v[pl.ds(pl.multiple_of(h * Dh, Dh), Dh), :]
        return attn + _mm(o_h.astype(bf16), w)

    attn = lax.fori_loop(0, H, head, jnp.zeros((_ROWS, D), f32))

    h1 = x + attn
    hn = _layernorm(h1)
    hn16 = hn.astype(bf16)
    wr = wr_v[...].astype(f32)
    racc = hn16[:, 0:128].astype(f32) * wr[0:1, :]
    for c in range(1, D // 128):
        racc = racc + hn16[:, c * 128:(c + 1) * 128].astype(f32) * wr[c:c + 1, :]
    gate_r = jax.nn.sigmoid(jnp.sum(racc, axis=-1, keepdims=True))
    wg_cp.wait()
    g = _mm(hn16, wg_v[...])
    g = g * jax.nn.sigmoid(g)
    wu_cp.wait()
    gu = (g * _mm(hn16, wu_v[...])).astype(bf16)
    wd_cp.wait()
    y = _mm(gu, wd_v[...]) * gate_r
    out = h1 + (hn + (hn * 0.0 + y))
    out_ref[...] = out[0:B, :].astype(out_ref.dtype)


@jax.jit
def pallas_sequential_preLN__mha_block_cached__moe_arch_mod__decode_kernel(
    A_x: jax.Array,
    A_k_cache: jax.Array,
    A_v_cache: jax.Array,
    A_wq: jax.Array,
    A_wo: jax.Array,
    B_x: jax.Array,
    B_w_r: jax.Array,
    B_w_gate: jax.Array,
    B_w_up: jax.Array,
    B_w_down: jax.Array,
):
    del B_x
    B, Sq, D = A_x.shape
    _, H, Sk, Dh = A_k_cache.shape
    F = B_w_gate.shape[1]
    assert Sq == 1 and D % 128 == 0 and B <= _ROWS and H % 2 == 0
    dt = A_k_cache.dtype
    hbm = pl.BlockSpec(memory_space=pl.ANY)
    out = pl.pallas_call(
        _kernel,
        out_shape=jax.ShapeDtypeStruct((B, D), A_x.dtype),
        in_specs=[hbm] * 9,
        out_specs=pl.BlockSpec(memory_space=pltpu.VMEM),
        scratch_shapes=[
            pltpu.VMEM((B, D), A_x.dtype),
            pltpu.VMEM((D, H * Dh), dt),
            pltpu.VMEM((H * Dh, D), dt),
            pltpu.VMEM((D // 128, 128), dt),
            pltpu.VMEM((D, F), dt),
            pltpu.VMEM((D, F), dt),
            pltpu.VMEM((F, D), dt),
            pltpu.VMEM((B, Dh, Sk), dt),
            pltpu.VMEM((B, Dh, Sk), dt),
            pltpu.VMEM((H, _ROWS, Dh), jnp.float32),
            pltpu.VMEM((_ROWS, D), jnp.float32),
            pltpu.SemaphoreType.DMA((B,)),
            pltpu.SemaphoreType.DMA((B,)),
            pltpu.SemaphoreType.DMA((7,)),
        ],
        compiler_params=pltpu.CompilerParams(vmem_limit_bytes=100 * 2**20),
    )(
        A_x.reshape(B, D),
        jnp.swapaxes(A_k_cache, 2, 3),
        jnp.swapaxes(A_v_cache, 2, 3),
        A_wq,
        A_wo,
        B_w_r.reshape(D // 128, 128),
        B_w_gate,
        B_w_up,
        B_w_down,
    )
    return out.reshape(B, Sq, D)
```

```python
import jax
import jax.numpy as jnp
from jax import lax
from jax.experimental import pallas as pl
from jax.experimental.pallas import tpu as pltpu

_EPS = 1e-5
_ROWS = 8
_SLOTS = 3
_KV_COLS = 256
_WIDE = (640,6144)
_TALL = (6144,640)


def _layernorm(x):
    m = jnp.mean(x, axis=-1, keepdims=True)
    d = x - m
    v = jnp.mean(d * d, axis=-1, keepdims=True)
    return d / jnp.sqrt(v + _EPS)


def _mm(a, b):
    return jnp.dot(a, b, preferred_element_type=jnp.float32)


def _start_tiled(src, dst, sem, tile):
    rows, cols = src.shape
    tr, tc = tile
    i = 0
    for r in range(0, rows, tr):
        for c in range(0, cols, tc):
            win = (pl.ds(r, min(tr, rows - r)), pl.ds(c, min(tc, cols - c)))
            pltpu.make_async_copy(src.at[win], dst.at[win], sem).start(priority=i % 2)
            i += 1


def _wait_all(dst, sem):
    pltpu.make_async_copy(dst, dst, sem).wait()


def _kernel(x_hbm, kt_hbm, vt_hbm, wq_hbm, wo_hbm, wr_hbm, wg_hbm, wu_hbm, wd_hbm,
            out_ref,
            x_v, wq_v, wo_v, wr_v, wg_v, wu_v, wd_v, k_buf, v_buf, q_s, xpad_s, o_s, attn_s,
            k_sem, v_sem, w_sem):
    f32, bf16 = jnp.float32, jnp.bfloat16
    B, H, Dh, _ = kt_hbm.shape
    D = x_hbm.shape[1]
    n_units = B * H
    scale = float(Dh) ** -0.5
    sem_x, sem_q, sem_o, sem_r, sem_g, sem_u, sem_d = (w_sem.at[i] for i in range(7))

    def start_kv(src, buf, sem, u):
        slot = u % _SLOTS
        _start_tiled(src.at[u % B, u // B], buf.at[slot], sem.at[slot], (Dh, _KV_COLS))

    x_cp = pltpu.make_async_copy(x_hbm, x_v, sem_x)
    wr_cp = pltpu.make_async_copy(wr_hbm, wr_v, sem_r)

    _start_tiled(wq_hbm, wq_v, sem_q, _WIDE)
    x_cp.start()
    wr_cp.start()
    start_kv(kt_hbm, k_buf, k_sem, 0)
    start_kv(vt_hbm, v_buf, v_sem, 0)

    x_cp.wait()
    wr_cp.wait()
    xpad_s[...] = jnp.zeros((_ROWS, D), f32)
    xpad_s[0:B, :] = x_v[...].astype(f32)
    xn = _layernorm(xpad_s[...]).astype(bf16)
    attn_s[...] = jnp.zeros((_ROWS, D), f32)
    o_s[...] = jnp.zeros((_ROWS, Dh), f32)
    _wait_all(wq_v, sem_q)

    @pl.loop(0, H // 2)
    def _(hp):
        q2 = _mm(xn, wq_v[:, pl.ds(pl.multiple_of(hp * 2 * Dh, 2 * Dh), 2 * Dh)])
        q_s[2 * hp] = q2[:, :Dh]
        q_s[2 * hp + 1] = q2[:, Dh:]

    @pl.loop(1, _SLOTS)
    def _(u):
        start_kv(kt_hbm, k_buf, k_sem, u)
        start_kv(vt_hbm, v_buf, v_sem, u)

    _start_tiled(wo_hbm, wo_v, sem_o, _TALL)

    @pl.loop(0, n_units)
    def _(u):
        h, b, slot = u // B, u % B, u % _SLOTS
        more = u + _SLOTS < n_units
        _wait_all(k_buf.at[slot], k_sem.at[slot])
        s = _mm(q_s[h].astype(bf16), k_buf[slot]) * scale
        p = jnp.exp(s - jnp.max(s, axis=-1, keepdims=True))
        l = jnp.sum(p, axis=-1, keepdims=True)

        @pl.when(more)
        def _():
            start_kv(kt_hbm, k_buf, k_sem, u + _SLOTS)

        _wait_all(v_buf.at[slot], v_sem.at[slot])
        o = lax.dot_general(p.astype(bf16), v_buf[slot], (((1,), (1,)), ((), ())),
                            preferred_element_type=f32)
        row = lax.broadcasted_iota(jnp.int32, (_ROWS, Dh), 0)
        o_s[...] = jnp.where(row == b, o / l, o_s[...])

        @pl.when(more)
        def _():
            start_kv(vt_hbm, v_buf, v_sem, u + _SLOTS)

        @pl.when(u == n_units - _SLOTS - 1)
        def _():
            _start_tiled(wg_hbm, wg_v, sem_g, _WIDE)
            _start_tiled(wu_hbm, wu_v, sem_u, _WIDE)
            _start_tiled(wd_hbm, wd_v, sem_d, _TALL)

        @pl.when(u == B - 1)
        def _():
            _wait_all(wo_v, sem_o)

        @pl.when(b == B - 1)
        def _():
            w = wo_v[pl.ds(pl.multiple_of(h * Dh, Dh), Dh), :]
            attn_s[...] += _mm(o_s[...].astype(bf16), w)

    h1 = xpad_s[...] + attn_s[...]
    hn = _layernorm(h1)
    hn16 = hn.astype(bf16)
    wr = wr_v[...].astype(f32)
    racc = hn16[:, 0:128].astype(f32) * wr[0:1, :]
    for c in range(1, D // 128):
        racc = racc + hn16[:, c * 128:(c + 1) * 128].astype(f32) * wr[c:c + 1, :]
    gate_r = jax.nn.sigmoid(jnp.sum(racc, axis=-1, keepdims=True))
    _wait_all(wg_v, sem_g)
    g = _mm(hn16, wg_v[...])
    g = g * jax.nn.sigmoid(g)
    _wait_all(wu_v, sem_u)
    gu = (g * _mm(hn16, wu_v[...])).astype(bf16)
    _wait_all(wd_v, sem_d)
    y = _mm(gu, wd_v[...]) * gate_r
    out = h1 + (hn + (hn * 0.0 + y))
    out_ref[...] = out[0:B, :].astype(out_ref.dtype)


@jax.jit
def pallas_sequential_preLN__mha_block_cached__moe_arch_mod__decode_kernel(
    A_x: jax.Array,
    A_k_cache: jax.Array,
    A_v_cache: jax.Array,
    A_wq: jax.Array,
    A_wo: jax.Array,
    B_x: jax.Array,
    B_w_r: jax.Array,
    B_w_gate: jax.Array,
    B_w_up: jax.Array,
    B_w_down: jax.Array,
):
    del B_x
    B, Sq, D = A_x.shape
    _, H, Sk, Dh = A_k_cache.shape
    F = B_w_gate.shape[1]
    assert Sq == 1 and D % 128 == 0 and B <= _ROWS and H % 2 == 0
    dt = A_k_cache.dtype
    hbm = pl.BlockSpec(memory_space=pl.ANY)
    out = pl.pallas_call(
        _kernel,
        out_shape=jax.ShapeDtypeStruct((B, D), A_x.dtype),
        in_specs=[hbm] * 9,
        out_specs=pl.BlockSpec(memory_space=pltpu.VMEM),
        scratch_shapes=[
            pltpu.VMEM((B, D), A_x.dtype),
            pltpu.VMEM((D, H * Dh), dt),
            pltpu.VMEM((H * Dh, D), dt),
            pltpu.VMEM((D // 128, 128), dt),
            pltpu.VMEM((D, F), dt),
            pltpu.VMEM((D, F), dt),
            pltpu.VMEM((F, D), dt),
            pltpu.VMEM((_SLOTS, Dh, Sk), dt),
            pltpu.VMEM((_SLOTS, Dh, Sk), dt),
            pltpu.VMEM((H, _ROWS, Dh), jnp.float32),
            pltpu.VMEM((_ROWS, D), jnp.float32),
            pltpu.VMEM((_ROWS, Dh), jnp.float32),
            pltpu.VMEM((_ROWS, D), jnp.float32),
            pltpu.SemaphoreType.DMA((_SLOTS,)),
            pltpu.SemaphoreType.DMA((_SLOTS,)),
            pltpu.SemaphoreType.DMA((7,)),
        ],
        compiler_params=pltpu.CompilerParams(vmem_limit_bytes=100 * 2**20),
    )(
        A_x.reshape(B, D),
        jnp.swapaxes(A_k_cache, 2, 3),
        jnp.swapaxes(A_v_cache, 2, 3),
        A_wq,
        A_wo,
        B_w_r.reshape(D // 128, 128),
        B_w_gate,
        B_w_up,
        B_w_down,
    )
    return out.reshape(B, Sq, D)
```

```python
import jax
import jax.numpy as jnp
from jax import lax
from jax.experimental import pallas as pl
from jax.experimental.pallas import tpu as pltpu

_EPS = 1e-5
_ROWS = 8
_TAIL = (2, 2, 2)
_SLOTS = 2
_KV_COLS = 256
_CHUNK = 2048
_WIDE = (160, 256)
_TALL = (64, 640)
_FCHUNK = 512


def _layernorm(x):
    m = jnp.mean(x, axis=-1, keepdims=True)
    d = x - m
    v = jnp.mean(d * d, axis=-1, keepdims=True)
    return d / jnp.sqrt(v + _EPS)


def _mm(a, b):
    return jnp.dot(a, b, preferred_element_type=jnp.float32)


def _ds(i, size):
    return pl.ds(pl.multiple_of(i * size, size), size)


def _start_tiled(src, dst, sem, tile):
    rows, cols = src.shape
    tr, tc = tile
    nr, nc = rows // tr, cols // tc
    assert nr * tr == rows and nc * tc == cols

    def start(r, c, queue):
        win = (_ds(r, tr) if nr > 1 else slice(None), _ds(c, tc) if nc > 1 else slice(None))
        pltpu.make_async_copy(src.at[win], dst.at[win], sem).start(priority=queue)

    if nc == 1:
        @pl.loop(0, nr // 2)
        def _(i):
            start(2 * i, 0, 0)
            start(2 * i + 1, 0, 1)
    else:
        @pl.loop(0, nr)
        def _(r):
            @pl.loop(0, nc // 2)
            def _(i):
                start(r, 2 * i, 0)
                start(r, 2 * i + 1, 1)


def _wait_all(dst, sem):
    pltpu.make_async_copy(dst, dst, sem).wait()


def _kernel(x_hbm, kt_hbm, vt_hbm, wq_hbm, wo_hbm, wr_hbm, wg_hbm, wu_hbm, wd_hbm,
            out_ref,
            x_v, wq_v, wo_v, wr_v, wg_v, wu_v, wd_v, k_buf, v_buf, q_s, xpad_s, attn_s, s_s, g_s,
            k_sem, v_sem, w_sem):
    f32, bf16 = jnp.float32, jnp.bfloat16
    B, H, Dh, Sk = kt_hbm.shape
    D = x_hbm.shape[1]
    F = wg_hbm.shape[1]
    n_units = B * H
    scale = float(Dh) ** -0.5
    sem_x, sem_q, sem_o, sem_r, sem_g, sem_u, sem_d = (w_sem.at[i] for i in range(7))

    def start_kv(src, buf, sem, u):
        slot = u % _SLOTS
        _start_tiled(src.at[u // H, u % H], buf.at[slot], sem.at[slot], (Dh, _KV_COLS))

    x_cp = pltpu.make_async_copy(x_hbm, x_v, sem_x)
    wr_cp = pltpu.make_async_copy(wr_hbm, wr_v, sem_r)

    _start_tiled(wq_hbm, wq_v, sem_q, _WIDE)
    x_cp.start()
    wr_cp.start()
    _start_tiled(wo_hbm, wo_v, sem_o, _TALL)

    x_cp.wait()
    wr_cp.wait()
    xpad_s[...] = jnp.zeros((_ROWS, D), f32)
    xpad_s[0:B, :] = x_v[...].astype(f32)
    xn = _layernorm(xpad_s[...]).astype(bf16)
    attn_s[...] = jnp.zeros((_ROWS, D), f32)
    _wait_all(wq_v, sem_q)

    @pl.loop(0, H // 2)
    def _(hp):
        q2 = _mm(xn, wq_v[:, _ds(hp, 2 * Dh)])
        q_s[2 * hp] = q2[:, :Dh]
        q_s[2 * hp + 1] = q2[:, Dh:]

    @pl.loop(0, _SLOTS)
    def _(u):
        start_kv(kt_hbm, k_buf, k_sem, u)
        start_kv(vt_hbm, v_buf, v_sem, u)

    _wait_all(wo_v, sem_o)

    @pl.loop(0, n_units)
    def _(u):
        b, h, slot = u // H, u % H, u % _SLOTS
        more = u + _SLOTS < n_units
        q = q_s[h].astype(bf16)
        _wait_all(k_buf.at[slot], k_sem.at[slot])

        def qk(c, m):
            s = _mm(q, k_buf[slot, :, _ds(c, _CHUNK)]) * scale
            s_s[:, _ds(c, _CHUNK)] = s
            for j in range(_CHUNK // 128):
                m = jnp.maximum(m, s[:, j * 128:(j + 1) * 128])
            return m

        m = lax.fori_loop(0, Sk // _CHUNK, qk, jnp.full((_ROWS, 128), -jnp.inf, f32))
        m = jnp.max(m, axis=-1, keepdims=True)

        @pl.when(more)
        def _():
            start_kv(kt_hbm, k_buf, k_sem, u + _SLOTS)

        @pl.when(u == n_units - _TAIL[0])
        def _():
            _start_tiled(wg_hbm, wg_v, sem_g, _WIDE)

        _wait_all(v_buf.at[slot], v_sem.at[slot])

        def pv(c, carry):
            l, o = carry
            p = jnp.exp(s_s[:, _ds(c, _CHUNK)] - m)
            for j in range(_CHUNK // 128):
                l = l + p[:, j * 128:(j + 1) * 128]
            o = o + lax.dot_general(p.astype(bf16), v_buf[slot, :, _ds(c, _CHUNK)],
                                    (((1,), (1,)), ((), ())), preferred_element_type=f32)
            return l, o

        l, o = lax.fori_loop(0, Sk // _CHUNK, pv,
                             (jnp.zeros((_ROWS, 128), f32), jnp.zeros((_ROWS, Dh), f32)))
        o = (o / jnp.sum(l, axis=-1, keepdims=True)).astype(bf16)
        attn = attn_s[...]
        proj = _mm(o, wo_v[_ds(h, Dh), :])
        row = lax.broadcasted_iota(jnp.int32, (_ROWS, D), 0)
        attn_s[...] = jnp.where(row == b, attn + proj, attn)

        @pl.when(more)
        def _():
            start_kv(vt_hbm, v_buf, v_sem, u + _SLOTS)

        @pl.when(u == n_units - _TAIL[1])
        def _():
            _start_tiled(wu_hbm, wu_v, sem_u, _WIDE)

        @pl.when(u == n_units - _TAIL[2])
        def _():
            _start_tiled(wd_hbm, wd_v, sem_d, _TALL)

    h1 = xpad_s[...] + attn_s[...]
    hn = _layernorm(h1)
    hn16 = hn.astype(bf16)
    wr = wr_v[...].astype(f32)
    racc = hn16[:, 0:128].astype(f32) * wr[0:1, :]
    for c in range(1, D // 128):
        racc = racc + hn16[:, c * 128:(c + 1) * 128].astype(f32) * wr[c:c + 1, :]
    gate_r = jax.nn.sigmoid(jnp.sum(racc, axis=-1, keepdims=True))
    _wait_all(wg_v, sem_g)

    @pl.loop(0, F // _FCHUNK)
    def _(c):
        g = _mm(hn16, wg_v[:, _ds(c, _FCHUNK)])
        g_s[:, _ds(c, _FCHUNK)] = g * jax.nn.sigmoid(g)

    _wait_all(wu_v, sem_u)

    @pl.loop(0, F // _FCHUNK)
    def _(c):
        g_s[:, _ds(c, _FCHUNK)] = g_s[:, _ds(c, _FCHUNK)] * _mm(hn16, wu_v[:, _ds(c, _FCHUNK)])

    _wait_all(wd_v, sem_d)

    def down(c, y):
        return y + _mm(g_s[:, _ds(c, _FCHUNK)].astype(bf16), wd_v[_ds(c, _FCHUNK), :])

    y = lax.fori_loop(0, F // _FCHUNK, down, jnp.zeros((_ROWS, D), f32)) * gate_r
    out = h1 + (hn + (hn * 0.0 + y))
    out_ref[...] = out[0:B, :].astype(out_ref.dtype)


@jax.jit
def pallas_sequential_preLN__mha_block_cached__moe_arch_mod__decode_kernel(
    A_x: jax.Array,
    A_k_cache: jax.Array,
    A_v_cache: jax.Array,
    A_wq: jax.Array,
    A_wo: jax.Array,
    B_x: jax.Array,
    B_w_r: jax.Array,
    B_w_gate: jax.Array,
    B_w_up: jax.Array,
    B_w_down: jax.Array,
):
    del B_x
    B, Sq, D = A_x.shape
    _, H, Sk, Dh = A_k_cache.shape
    F = B_w_gate.shape[1]
    assert Sq == 1 and D % 128 == 0 and B <= _ROWS and H % 2 == 0
    dt = A_k_cache.dtype
    hbm = pl.BlockSpec(memory_space=pl.ANY)
    out = pl.pallas_call(
        _kernel,
        out_shape=jax.ShapeDtypeStruct((B, D), A_x.dtype),
        in_specs=[hbm] * 9,
        out_specs=pl.BlockSpec(memory_space=pltpu.VMEM),
        scratch_shapes=[
            pltpu.VMEM((B, D), A_x.dtype),
            pltpu.VMEM((D, H * Dh), dt),
            pltpu.VMEM((H * Dh, D), dt),
            pltpu.VMEM((D // 128, 128), dt),
            pltpu.VMEM((D, F), dt),
            pltpu.VMEM((D, F), dt),
            pltpu.VMEM((F, D), dt),
            pltpu.VMEM((_SLOTS, Dh, Sk), dt),
            pltpu.VMEM((_SLOTS, Dh, Sk), dt),
            pltpu.VMEM((H, _ROWS, Dh), jnp.float32),
            pltpu.VMEM((_ROWS, D), jnp.float32),
            pltpu.VMEM((_ROWS, D), jnp.float32),
            pltpu.VMEM((_ROWS, Sk), jnp.float32),
            pltpu.VMEM((_ROWS, F), jnp.float32),
            pltpu.SemaphoreType.DMA((_SLOTS,)),
            pltpu.SemaphoreType.DMA((_SLOTS,)),
            pltpu.SemaphoreType.DMA((7,)),
        ],
        compiler_params=pltpu.CompilerParams(vmem_limit_bytes=100 * 2**20),
    )(
        A_x.reshape(B, D),
        jnp.swapaxes(A_k_cache, 2, 3),
        jnp.swapaxes(A_v_cache, 2, 3),
        A_wq,
        A_wo,
        B_w_r.reshape(D // 128, 128),
        B_w_gate,
        B_w_up,
        B_w_down,
    )
    return out.reshape(B, Sq, D)
```

```python
import jax
import jax.numpy as jnp
from jax import lax
from jax.experimental import pallas as pl
from jax.experimental.pallas import tpu as pltpu

_EPS = 1e-5
_ROWS = 8
_TAIL = (2, 2, 2)
_SLOTS = 2
_KV_COLS = 256
_CHUNK = 2048
_WIDE = (160, 256)
_TALL = (64, 640)
_FCHUNK = 512
_DCHUNK = 256


def _layernorm(x):
    m = jnp.mean(x, axis=-1, keepdims=True)
    d = x - m
    v = jnp.mean(d * d, axis=-1, keepdims=True)
    return d / jnp.sqrt(v + _EPS)


def _mm(a, b):
    return jnp.dot(a, b, preferred_element_type=jnp.float32)


def _ds(i, size):
    return pl.ds(pl.multiple_of(i * size, size), size)


def _start_tiled(src, dst, sem, tile):
    rows, cols = src.shape
    tr, tc = tile
    nr, nc = rows // tr, cols // tc
    assert nr * tr == rows and nc * tc == cols

    def start(r, c, queue):
        win = (_ds(r, tr) if nr > 1 else slice(None), _ds(c, tc) if nc > 1 else slice(None))
        pltpu.make_async_copy(src.at[win], dst.at[win], sem).start(priority=queue)

    if nc == 1:
        @pl.loop(0, nr // 2)
        def _(i):
            start(2 * i, 0, 0)
            start(2 * i + 1, 0, 1)
    else:
        @pl.loop(0, nr)
        def _(r):
            @pl.loop(0, nc // 2)
            def _(i):
                start(r, 2 * i, 0)
                start(r, 2 * i + 1, 1)


def _wait_all(dst, sem):
    pltpu.make_async_copy(dst, dst, sem).wait()


def _kernel(x_hbm, kt_hbm, vt_hbm, wq_hbm, wo_hbm, wr_hbm, wg_hbm, wu_hbm, wd_hbm,
            out_ref,
            x_v, wq_v, wo_v, wr_v, wg_v, wu_v, wd_v, k_buf, v_buf, q_s, xpad_s, attn_s, s_s, g_s,
            k_sem, v_sem, w_sem, d_sem):
    f32, bf16 = jnp.float32, jnp.bfloat16
    B, H, Dh, Sk = kt_hbm.shape
    D = x_hbm.shape[1]
    F = wg_hbm.shape[1]
    n_units = B * H
    scale = float(Dh) ** -0.5
    sem_x, sem_q, sem_o, sem_r, sem_g, sem_u = (w_sem.at[i] for i in range(6))

    def start_kv(src, buf, sem, u):
        slot = u % _SLOTS
        _start_tiled(src.at[u // H, u % H], buf.at[slot], sem.at[slot], (Dh, _KV_COLS))

    x_cp = pltpu.make_async_copy(x_hbm, x_v, sem_x)
    wr_cp = pltpu.make_async_copy(wr_hbm, wr_v, sem_r)

    _start_tiled(wq_hbm, wq_v, sem_q, _WIDE)
    x_cp.start()
    wr_cp.start()
    _start_tiled(wo_hbm, wo_v, sem_o, _TALL)

    x_cp.wait()
    wr_cp.wait()
    xpad_s[...] = jnp.zeros((_ROWS, D), f32)
    xpad_s[0:B, :] = x_v[...].astype(f32)
    xn = _layernorm(xpad_s[...]).astype(bf16)
    attn_s[...] = jnp.zeros((_ROWS, D), f32)
    _wait_all(wq_v, sem_q)

    @pl.loop(0, H // 2)
    def _(hp):
        q2 = _mm(xn, wq_v[:, _ds(hp, 2 * Dh)])
        q_s[2 * hp] = q2[:, :Dh]
        q_s[2 * hp + 1] = q2[:, Dh:]

    @pl.loop(0, _SLOTS)
    def _(u):
        start_kv(kt_hbm, k_buf, k_sem, u)
        start_kv(vt_hbm, v_buf, v_sem, u)

    _wait_all(wo_v, sem_o)

    @pl.loop(0, n_units)
    def _(u):
        b, h, slot = u // H, u % H, u % _SLOTS
        more = u + _SLOTS < n_units
        q = q_s[h].astype(bf16)
        _wait_all(k_buf.at[slot], k_sem.at[slot])

        def qk(c, m):
            s = _mm(q, k_buf[slot, :, _ds(c, _CHUNK)]) * scale
            s_s[:, _ds(c, _CHUNK)] = s
            for j in range(_CHUNK // 128):
                m = jnp.maximum(m, s[:, j * 128:(j + 1) * 128])
            return m

        m = lax.fori_loop(0, Sk // _CHUNK, qk, jnp.full((_ROWS, 128), -jnp.inf, f32))
        m = jnp.max(m, axis=-1, keepdims=True)

        @pl.when(more)
        def _():
            start_kv(kt_hbm, k_buf, k_sem, u + _SLOTS)

        @pl.when(u == n_units - _TAIL[0])
        def _():
            pltpu.make_async_copy(wg_hbm, wg_v, sem_g).start(priority=1)

        _wait_all(v_buf.at[slot], v_sem.at[slot])

        def pv(c, carry):
            l, o = carry
            p = jnp.exp(s_s[:, _ds(c, _CHUNK)] - m)
            for j in range(_CHUNK // 128):
                l = l + p[:, j * 128:(j + 1) * 128]
            o = o + lax.dot_general(p.astype(bf16), v_buf[slot, :, _ds(c, _CHUNK)],
                                    (((1,), (1,)), ((), ())), preferred_element_type=f32)
            return l, o

        l, o = lax.fori_loop(0, Sk // _CHUNK, pv,
                             (jnp.zeros((_ROWS, 128), f32), jnp.zeros((_ROWS, Dh), f32)))
        o = (o / jnp.sum(l, axis=-1, keepdims=True)).astype(bf16)
        attn = attn_s[...]
        proj = _mm(o, wo_v[_ds(h, Dh), :])
        row = lax.broadcasted_iota(jnp.int32, (_ROWS, D), 0)
        attn_s[...] = jnp.where(row == b, attn + proj, attn)

        @pl.when(more)
        def _():
            start_kv(vt_hbm, v_buf, v_sem, u + _SLOTS)

        @pl.when(u == n_units - _TAIL[1])
        def _():
            pltpu.make_async_copy(wu_hbm, wu_v, sem_u).start(priority=1)

        @pl.when(u == n_units - _TAIL[2])
        def _():
            @pl.loop(0, F // _DCHUNK)
            def _(c):
                rows = _ds(c, _DCHUNK)
                pltpu.make_async_copy(wd_hbm.at[rows], wd_v.at[rows], d_sem.at[c]).start(priority=1)

    h1 = xpad_s[...] + attn_s[...]
    hn = _layernorm(h1)
    hn16 = hn.astype(bf16)
    wr = wr_v[...].astype(f32)
    racc = hn16[:, 0:128].astype(f32) * wr[0:1, :]
    for c in range(1, D // 128):
        racc = racc + hn16[:, c * 128:(c + 1) * 128].astype(f32) * wr[c:c + 1, :]
    gate_r = jax.nn.sigmoid(jnp.sum(racc, axis=-1, keepdims=True))
    _wait_all(wg_v, sem_g)

    @pl.loop(0, F // _FCHUNK)
    def _(c):
        g = _mm(hn16, wg_v[:, _ds(c, _FCHUNK)])
        g_s[:, _ds(c, _FCHUNK)] = g * jax.nn.sigmoid(g)

    _wait_all(wu_v, sem_u)

    @pl.loop(0, F // _FCHUNK)
    def _(c):
        g_s[:, _ds(c, _FCHUNK)] = g_s[:, _ds(c, _FCHUNK)] * _mm(hn16, wu_v[:, _ds(c, _FCHUNK)])

    def down(c, y):
        rows = _ds(c, _DCHUNK)
        _wait_all(wd_v.at[rows], d_sem.at[c])
        return y + _mm(g_s[:, rows].astype(bf16), wd_v[rows, :])

    y = lax.fori_loop(0, F // _DCHUNK, down, jnp.zeros((_ROWS, D), f32)) * gate_r
    out = h1 + (hn + (hn * 0.0 + y))
    out_ref[...] = out[0:B, :].astype(out_ref.dtype)


@jax.jit
def pallas_sequential_preLN__mha_block_cached__moe_arch_mod__decode_kernel(
    A_x: jax.Array,
    A_k_cache: jax.Array,
    A_v_cache: jax.Array,
    A_wq: jax.Array,
    A_wo: jax.Array,
    B_x: jax.Array,
    B_w_r: jax.Array,
    B_w_gate: jax.Array,
    B_w_up: jax.Array,
    B_w_down: jax.Array,
):
    del B_x
    B, Sq, D = A_x.shape
    _, H, Sk, Dh = A_k_cache.shape
    F = B_w_gate.shape[1]
    assert Sq == 1 and D % 128 == 0 and B <= _ROWS and H % 2 == 0
    dt = A_k_cache.dtype
    hbm = pl.BlockSpec(memory_space=pl.ANY)
    out = pl.pallas_call(
        _kernel,
        out_shape=jax.ShapeDtypeStruct((B, D), A_x.dtype),
        in_specs=[hbm] * 9,
        out_specs=pl.BlockSpec(memory_space=pltpu.VMEM),
        scratch_shapes=[
            pltpu.VMEM((B, D), A_x.dtype),
            pltpu.VMEM((D, H * Dh), dt),
            pltpu.VMEM((H * Dh, D), dt),
            pltpu.VMEM((D // 128, 128), dt),
            pltpu.VMEM((D, F), dt),
            pltpu.VMEM((D, F), dt),
            pltpu.VMEM((F, D), dt),
            pltpu.VMEM((_SLOTS, Dh, Sk), dt),
            pltpu.VMEM((_SLOTS, Dh, Sk), dt),
            pltpu.VMEM((H, _ROWS, Dh), jnp.float32),
            pltpu.VMEM((_ROWS, D), jnp.float32),
            pltpu.VMEM((_ROWS, D), jnp.float32),
            pltpu.VMEM((_ROWS, Sk), jnp.float32),
            pltpu.VMEM((_ROWS, F), jnp.float32),
            pltpu.SemaphoreType.DMA((_SLOTS,)),
            pltpu.SemaphoreType.DMA((_SLOTS,)),
            pltpu.SemaphoreType.DMA((6,)),
            pltpu.SemaphoreType.DMA((F // _DCHUNK,)),
        ],
        compiler_params=pltpu.CompilerParams(vmem_limit_bytes=100 * 2**20),
    )(
        A_x.reshape(B, D),
        jnp.swapaxes(A_k_cache, 2, 3),
        jnp.swapaxes(A_v_cache, 2, 3),
        A_wq,
        A_wo,
        B_w_r.reshape(D // 128, 128),
        B_w_gate,
        B_w_up,
        B_w_down,
    )
    return out.reshape(B, Sq, D)
```

```python
import jax
import jax.numpy as jnp
from jax import lax
from jax.experimental import pallas as pl
from jax.experimental.pallas import tpu as pltpu

_EPS = 1e-5
_ROWS = 8
_SLOTS = 2
_KV_COLS = 256
_CHUNK = 2048
_WIDE = (160, 256)
_TALL_ROWS = 64
_FCHUNK = 512
_DCHUNK = 256


def _layernorm(x):
    m = jnp.mean(x, axis=-1, keepdims=True)
    d = x - m
    v = jnp.mean(d * d, axis=-1, keepdims=True)
    return d / jnp.sqrt(v + _EPS)


def _mm(a, b):
    return jnp.dot(a, b, preferred_element_type=jnp.float32)


def _ds(i, size):
    return pl.ds(pl.multiple_of(i * size, size), size)


def _start_tiled(src, dst, sem, tile):
    rows, cols = src.shape
    tr, tc = tile
    nr, nc = rows // tr, cols // tc
    assert nr * tr == rows and nc * tc == cols and (nr if nc == 1 else nc) % 2 == 0

    def start(r, c, queue):
        win = (_ds(r, tr) if nr > 1 else slice(None), _ds(c, tc) if nc > 1 else slice(None))
        pltpu.make_async_copy(src.at[win], dst.at[win], sem).start(priority=queue)

    if nc == 1:
        @pl.loop(0, nr // 2)
        def _(i):
            start(2 * i, 0, 0)
            start(2 * i + 1, 0, 1)
    else:
        @pl.loop(0, nr)
        def _(r):
            @pl.loop(0, nc // 2)
            def _(i):
                start(r, 2 * i, 0)
                start(r, 2 * i + 1, 1)


def _wait_all(dst, sem):
    pltpu.make_async_copy(dst, dst, sem).wait()


def _kernel(x_hbm, kt_hbm, vt_hbm, wq_hbm, wo_hbm, wr_hbm, wg_hbm, wu_hbm, wd_hbm,
            out_ref,
            x_v, wq_v, wo_v, wr_v, wg_v, wu_v, wd_v, k_buf, v_buf,
            q_s, xpad_s, attn_s, s_s, g_s,
            k_sem, v_sem, w_sem, d_sem):
    f32, bf16 = jnp.float32, jnp.bfloat16
    B, H, Dh, Sk = kt_hbm.shape
    D = x_hbm.shape[1]
    F = wg_hbm.shape[1]
    n_units = B * H
    scale = float(Dh) ** -0.5
    sem_x, sem_q, sem_o, sem_r, sem_g, sem_u = (w_sem.at[i] for i in range(6))

    def start_kv(src, buf, sem, u):
        slot = u % _SLOTS
        _start_tiled(src.at[u // H, u % H], buf.at[slot], sem.at[slot], (Dh, _KV_COLS))

    def wd_cp(c):
        rows = _ds(c, _DCHUNK)
        return pltpu.make_async_copy(wd_hbm.at[rows], wd_v.at[rows], d_sem.at[c])

    x_cp = pltpu.make_async_copy(x_hbm, x_v, sem_x)
    wr_cp = pltpu.make_async_copy(wr_hbm, wr_v, sem_r)

    _start_tiled(wq_hbm, wq_v, sem_q, _WIDE)
    x_cp.start()
    wr_cp.start()
    _start_tiled(wo_hbm, wo_v, sem_o, (_TALL_ROWS, D))

    x_cp.wait()
    wr_cp.wait()
    xpad_s[...] = jnp.zeros((_ROWS, D), f32)
    xpad_s[0:B, :] = x_v[...].astype(f32)
    xn = _layernorm(xpad_s[...]).astype(bf16)
    attn_s[...] = jnp.zeros((_ROWS, D), f32)
    _wait_all(wq_v, sem_q)

    @pl.loop(0, H // 2)
    def _(hp):
        q2 = _mm(xn, wq_v[:, _ds(hp, 2 * Dh)])
        q_s[2 * hp] = q2[:, :Dh]
        q_s[2 * hp + 1] = q2[:, Dh:]

    @pl.loop(0, _SLOTS)
    def _(u):
        start_kv(kt_hbm, k_buf, k_sem, u)
        start_kv(vt_hbm, v_buf, v_sem, u)

    _wait_all(wo_v, sem_o)

    @pl.loop(0, n_units)
    def _(u):
        b, h, slot = u // H, u % H, u % _SLOTS
        more = u + _SLOTS < n_units
        kv_all_requested = u + _SLOTS == n_units
        q = q_s[h].astype(bf16)
        _wait_all(k_buf.at[slot], k_sem.at[slot])

        def qk(c, m):
            s = _mm(q, k_buf[slot, :, _ds(c, _CHUNK)]) * scale
            s_s[:, _ds(c, _CHUNK)] = s
            for j in range(_CHUNK // 128):
                m = jnp.maximum(m, s[:, j * 128:(j + 1) * 128])
            return m

        m = lax.fori_loop(0, Sk // _CHUNK, qk, jnp.full((_ROWS, 128), -jnp.inf, f32))
        m = jnp.max(m, axis=-1, keepdims=True)

        @pl.when(more)
        def _():
            start_kv(kt_hbm, k_buf, k_sem, u + _SLOTS)

        @pl.when(kv_all_requested)
        def _():
            _start_tiled(wg_hbm, wg_v, sem_g, _WIDE)

        _wait_all(v_buf.at[slot], v_sem.at[slot])

        def pv(c, carry):
            l, o = carry
            p = jnp.exp(s_s[:, _ds(c, _CHUNK)] - m)
            for j in range(_CHUNK // 128):
                l = l + p[:, j * 128:(j + 1) * 128]
            o = o + lax.dot_general(p.astype(bf16), v_buf[slot, :, _ds(c, _CHUNK)],
                                    (((1,), (1,)), ((), ())), preferred_element_type=f32)
            return l, o

        l, o = lax.fori_loop(0, Sk // _CHUNK, pv,
                             (jnp.zeros((_ROWS, 128), f32), jnp.zeros((_ROWS, Dh), f32)))
        o = (o / jnp.sum(l, axis=-1, keepdims=True)).astype(bf16)
        attn = attn_s[...]
        proj = _mm(o, wo_v[_ds(h, Dh), :])
        row = lax.broadcasted_iota(jnp.int32, (_ROWS, D), 0)
        attn_s[...] = jnp.where(row == b, attn + proj, attn)

        @pl.when(more)
        def _():
            start_kv(vt_hbm, v_buf, v_sem, u + _SLOTS)

        @pl.when(kv_all_requested)
        def _():
            _start_tiled(wu_hbm, wu_v, sem_u, _WIDE)

            @pl.loop(0, F // _DCHUNK)
            def _(c):
                wd_cp(c).start(priority=1)

    h1 = xpad_s[...] + attn_s[...]
    hn = _layernorm(h1)
    hn16 = hn.astype(bf16)
    wr = wr_v[...].astype(f32)
    racc = hn16[:, 0:128].astype(f32) * wr[0:1, :]
    for c in range(1, D // 128):
        racc = racc + hn16[:, c * 128:(c + 1) * 128].astype(f32) * wr[c:c + 1, :]
    gate_r = jax.nn.sigmoid(jnp.sum(racc, axis=-1, keepdims=True))
    _wait_all(wg_v, sem_g)

    @pl.loop(0, F // _FCHUNK)
    def _(c):
        g = _mm(hn16, wg_v[:, _ds(c, _FCHUNK)])
        g_s[:, _ds(c, _FCHUNK)] = g * jax.nn.sigmoid(g)

    _wait_all(wu_v, sem_u)

    @pl.loop(0, F // _FCHUNK)
    def _(c):
        g_s[:, _ds(c, _FCHUNK)] = g_s[:, _ds(c, _FCHUNK)] * _mm(hn16, wu_v[:, _ds(c, _FCHUNK)])

    def down(c, y):
        rows = _ds(c, _DCHUNK)
        wd_cp(c).wait()
        return y + _mm(g_s[:, rows].astype(bf16), wd_v[rows, :])

    y = lax.fori_loop(0, F // _DCHUNK, down, jnp.zeros((_ROWS, D), f32)) * gate_r
    out = h1 + (hn + (hn * 0.0 + y))
    out_ref[...] = out[0:B, :].astype(out_ref.dtype)


@jax.jit
def pallas_sequential_preLN__mha_block_cached__moe_arch_mod__decode_kernel(
    A_x: jax.Array,
    A_k_cache: jax.Array,
    A_v_cache: jax.Array,
    A_wq: jax.Array,
    A_wo: jax.Array,
    B_x: jax.Array,
    B_w_r: jax.Array,
    B_w_gate: jax.Array,
    B_w_up: jax.Array,
    B_w_down: jax.Array,
):
    del B_x
    B, Sq, D = A_x.shape
    _, H, Sk, Dh = A_k_cache.shape
    F = B_w_gate.shape[1]
    assert Sq == 1 and D % 128 == 0 and B <= _ROWS and H % 2 == 0 and B * H >= _SLOTS
    assert Sk % _CHUNK == 0 and F % _FCHUNK == 0 and F % _DCHUNK == 0
    dt = A_k_cache.dtype
    hbm = pl.BlockSpec(memory_space=pl.ANY)
    out = pl.pallas_call(
        _kernel,
        out_shape=jax.ShapeDtypeStruct((B, D), A_x.dtype),
        in_specs=[hbm] * 9,
        out_specs=pl.BlockSpec(memory_space=pltpu.VMEM),
        scratch_shapes=[
            pltpu.VMEM((B, D), A_x.dtype),
            pltpu.VMEM((D, H * Dh), dt),
            pltpu.VMEM((H * Dh, D), dt),
            pltpu.VMEM((D // 128, 128), dt),
            pltpu.VMEM((D, F), dt),
            pltpu.VMEM((D, F), dt),
            pltpu.VMEM((F, D), dt),
            pltpu.VMEM((_SLOTS, Dh, Sk), dt),
            pltpu.VMEM((_SLOTS, Dh, Sk), dt),
            pltpu.VMEM((H, _ROWS, Dh), jnp.float32),
            pltpu.VMEM((_ROWS, D), jnp.float32),
            pltpu.VMEM((_ROWS, D), jnp.float32),
            pltpu.VMEM((_ROWS, Sk), jnp.float32),
            pltpu.VMEM((_ROWS, F), jnp.float32),
            pltpu.SemaphoreType.DMA((_SLOTS,)),
            pltpu.SemaphoreType.DMA((_SLOTS,)),
            pltpu.SemaphoreType.DMA((6,)),
            pltpu.SemaphoreType.DMA((F // _DCHUNK,)),
        ],
        compiler_params=pltpu.CompilerParams(vmem_limit_bytes=100 * 2**20),
    )(
        A_x.reshape(B, D),
        jnp.swapaxes(A_k_cache, 2, 3),
        jnp.swapaxes(A_v_cache, 2, 3),
        A_wq,
        A_wo,
        B_w_r.reshape(D // 128, 128),
        B_w_gate,
        B_w_up,
        B_w_down,
    )
    return out.reshape(B, Sq, D)
```
